```python
import os as _os
_os.environ.setdefault("JAX_PLATFORMS", "cpu")
import jax
import jax.numpy as jnp

def _softmax(x, axis=-1):
    return jax.nn.softmax(x, axis=axis)
def _gelu(x):
    return jax.nn.gelu(x, approximate=True)
def _silu(x):
    return jax.nn.silu(x)
def _sigmoid(x):
    return jax.nn.sigmoid(x)
def _layernorm(x, axis=-1, eps=1e-5):
    m = jnp.mean(x, axis=axis, keepdims=True)
    v = jnp.var(x, axis=axis, keepdims=True)
    return (x - m) / jnp.sqrt(v + eps)
def _scatter_add(tgt, idx, src, axis=0):
    return tgt.at[idx].add(src)
def _segment_sum(src, seg, n):
    return jax.ops.segment_sum(src, seg, n)
class _Rng:
    def __init__(self, key):
        self._k = key
    def _next(self):
        self._k, sub = jax.random.split(self._k)
        return sub
    def normal(self, shape):
        return jax.random.normal(self._next(), shape, dtype=jnp.bfloat16)
    def randint(self, lo, hi, shape):
        return jax.random.randint(self._next(), shape, lo, hi, dtype=jnp.int32)
    def uniform(self, shape, lo=0.0, hi=1.0):
        return jax.random.uniform(self._next(), shape, jnp.bfloat16, lo, hi)
    def permutation(self, n):
        return jax.random.permutation(self._next(), n)


kernel_name = 'standalone__mha_softmax__near_ridge'

def setup_inputs():
    _rng = _Rng(jax.random.key(int.from_bytes(__import__("os").urandom(4), "little")))
    _w = (lambda a: (lambda t: t.astype(jnp.bfloat16) if jnp.issubdtype(t.dtype, jnp.floating) else t)(jnp.asarray(a)))
    B, H, Sq, Sk, D = 8, 32, 304, 2048, 128
    return {
        "q": _w((lambda *s: _rng.normal(s) * 0.4)(B, H, Sq, D)),
        "k": _w((lambda *s: _rng.normal(s) * 0.4)(B, H, Sk, D)),
        "v": _w((lambda *s: _rng.normal(s) * 0.05)(B, H, Sk, D)),
    }

def reference(q, k, v):
    scale = q.shape[-1] ** -0.5
    scores = jnp.einsum("bhqd,bhkd->bhqk", q, k) * scale
    p = _softmax(scores, axis=-1)
    return jnp.einsum("bhqk,bhkd->bhqd", p, v)
```

```python
import functools
import math

import jax
import jax.numpy as jnp
import jax.experimental.pallas as pl
import jax.experimental.pallas.tpu as pltpu

HEADS_PER_STEP = 8
KV_CHUNK = 512


def _attention_kernel(q_ref, k_ref, v_ref, o_ref, *, scale, heads, sk):
    c = scale * math.log2(math.e)
    n_chunks = sk // KV_CHUNK
    trans_b = (((1,), (1,)), ((), ()))

    def scaled_q(h):
        return (q_ref[h].astype(jnp.float32) * c).astype(jnp.bfloat16)

    def scores(qh, h, g):
        kg = k_ref[h, g * KV_CHUNK:(g + 1) * KV_CHUNK, :]
        return jax.lax.dot_general(qh, kg, trans_b, preferred_element_type=jnp.float32)

    q0 = scaled_q(0)
    s_cur = [scores(q0, 0, g) for g in range(n_chunks)]
    for h in range(heads):
        m = jnp.max(functools.reduce(jnp.maximum, s_cur), axis=-1, keepdims=True)
        has_next = h + 1 < heads
        q_next = scaled_q(h + 1) if has_next else None
        s_next = []
        acc = None
        lsum = None
        for g in range(n_chunks):
            if has_next:
                s_next.append(scores(q_next, h + 1, g))
            p = jnp.exp2(s_cur[g] - m)
            lsum = p if lsum is None else lsum + p
            vg = v_ref[h, g * KV_CHUNK:(g + 1) * KV_CHUNK, :]
            o = jnp.dot(p.astype(jnp.bfloat16), vg, preferred_element_type=jnp.float32)
            acc = o if acc is None else acc + o
        l = jnp.sum(lsum, axis=-1, keepdims=True)
        r = pl.reciprocal(l, approx=True)
        r = r * (2.0 - l * r)
        o_ref[h] = (acc * r).astype(o_ref.dtype)
        s_cur = s_next


@jax.jit
def pallas_standalone__mha_softmax__near_ridge_kernel(q, k, v):
    B, H, Sq, D = q.shape
    Sk = k.shape[2]
    BH = B * H
    hb = HEADS_PER_STEP
    q3 = q.reshape(BH, Sq, D)
    k3 = k.reshape(BH, Sk, D)
    v3 = v.reshape(BH, Sk, D)
    out = pl.pallas_call(
        functools.partial(_attention_kernel, scale=D ** -0.5, heads=hb, sk=Sk),
        grid=(BH // hb,),
        in_specs=[
            pl.BlockSpec((hb, Sq, D), lambda i: (i, 0, 0)),
            pl.BlockSpec((hb, Sk, D), lambda i: (i, 0, 0)),
            pl.BlockSpec((hb, Sk, D), lambda i: (i, 0, 0)),
        ],
        out_specs=pl.BlockSpec((hb, Sq, D), lambda i: (i, 0, 0)),
        out_shape=jax.ShapeDtypeStruct((BH, Sq, D), q.dtype),
        compiler_params=pltpu.CompilerParams(
            dimension_semantics=("parallel",),
            vmem_limit_bytes=100 * 1024 * 1024,
        ),
    )(q3, k3, v3)
    return out.reshape(B, H, Sq, D)
```

```python
import functools
import math

import jax
import jax.numpy as jnp
import jax.experimental.pallas as pl
import jax.experimental.pallas.tpu as pltpu

HEADS_PER_STEP = 8
KV_CHUNK = 512
ROW_SPLITS = ((0, 96), (96, 192), (192, 304))


def _attention_kernel(q_ref, k_ref, v_ref, o_ref, *, scale, heads, sk):
    c = scale * math.log2(math.e)
    n_chunks = sk // KV_CHUNK
    trans_b = (((1,), (1,)), ((), ()))
    units = [(h, r0, r1) for h in range(heads) for (r0, r1) in ROW_SPLITS]

    def scaled_q(unit):
        h, r0, r1 = unit
        return (q_ref[h, r0:r1, :].astype(jnp.float32) * c).astype(jnp.bfloat16)

    def scores(qu, h, g):
        kg = k_ref[h, g * KV_CHUNK:(g + 1) * KV_CHUNK, :]
        return jax.lax.dot_general(qu, kg, trans_b, preferred_element_type=jnp.float32)

    s_cur = [scores(scaled_q(units[0]), units[0][0], g) for g in range(n_chunks)]
    for u, (h, r0, r1) in enumerate(units):
        m = jnp.max(functools.reduce(jnp.maximum, s_cur), axis=-1, keepdims=True)
        has_next = u + 1 < len(units)
        q_next = scaled_q(units[u + 1]) if has_next else None
        s_next = []
        acc = None
        lsum = None
        for g in range(n_chunks):
            if has_next:
                s_next.append(scores(q_next, units[u + 1][0], g))
            p = jnp.exp2(s_cur[g] - m)
            lsum = p if lsum is None else lsum + p
            vg = v_ref[h, g * KV_CHUNK:(g + 1) * KV_CHUNK, :]
            o = jnp.dot(p.astype(jnp.bfloat16), vg, preferred_element_type=jnp.float32)
            acc = o if acc is None else acc + o
        l = jnp.sum(lsum, axis=-1, keepdims=True)
        r = pl.reciprocal(l, approx=True)
        r = r * (2.0 - l * r)
        o_ref[h, r0:r1, :] = (acc * r).astype(o_ref.dtype)
        s_cur = s_next


@jax.jit
def pallas_standalone__mha_softmax__near_ridge_kernel(q, k, v):
    B, H, Sq, D = q.shape
    Sk = k.shape[2]
    BH = B * H
    hb = HEADS_PER_STEP
    q3 = q.reshape(BH, Sq, D)
    k3 = k.reshape(BH, Sk, D)
    v3 = v.reshape(BH, Sk, D)
    out = pl.pallas_call(
        functools.partial(_attention_kernel, scale=D ** -0.5, heads=hb, sk=Sk),
        grid=(BH // hb,),
        in_specs=[
            pl.BlockSpec((hb, Sq, D), lambda i: (i, 0, 0)),
            pl.BlockSpec((hb, Sk, D), lambda i: (i, 0, 0)),
            pl.BlockSpec((hb, Sk, D), lambda i: (i, 0, 0)),
        ],
        out_specs=pl.BlockSpec((hb, Sq, D), lambda i: (i, 0, 0)),
        out_shape=jax.ShapeDtypeStruct((BH, Sq, D), q.dtype),
        compiler_params=pltpu.CompilerParams(
            dimension_semantics=("parallel",),
            vmem_limit_bytes=100 * 1024 * 1024,
        ),
    )(q3, k3, v3)
    return out.reshape(B, H, Sq, D)
```
